```python
import os as _os
_os.environ.setdefault("JAX_PLATFORMS", "cpu")
import jax
import jax.numpy as jnp

def _softmax(x, axis=-1):
    return jax.nn.softmax(x, axis=axis)
def _gelu(x):
    return jax.nn.gelu(x, approximate=True)
def _silu(x):
    return jax.nn.silu(x)
def _sigmoid(x):
    return jax.nn.sigmoid(x)
def _layernorm(x, axis=-1, eps=1e-5):
    m = jnp.mean(x, axis=axis, keepdims=True)
    v = jnp.var(x, axis=axis, keepdims=True)
    return (x - m) / jnp.sqrt(v + eps)
def _scatter_add(tgt, idx, src, axis=0):
    return tgt.at[idx].add(src)
def _segment_sum(src, seg, n):
    return jax.ops.segment_sum(src, seg, n)
class _Rng:
    def __init__(self, key):
        self._k = key
    def _next(self):
        self._k, sub = jax.random.split(self._k)
        return sub
    def normal(self, shape):
        return jax.random.normal(self._next(), shape, dtype=jnp.bfloat16)
    def randint(self, lo, hi, shape):
        return jax.random.randint(self._next(), shape, lo, hi, dtype=jnp.int32)
    def uniform(self, shape, lo=0.0, hi=1.0):
        return jax.random.uniform(self._next(), shape, jnp.bfloat16, lo, hi)
    def permutation(self, n):
        return jax.random.permutation(self._next(), n)


kernel_name = 'standalone__glu_gated_bilinear__prompt'

def setup_inputs():
    _rng = _Rng(jax.random.key(int.from_bytes(__import__("os").urandom(4), "little")))
    _w = (lambda a: (lambda t: t.astype(jnp.bfloat16) if jnp.issubdtype(t.dtype, jnp.floating) else t)(jnp.asarray(a)))
    B, S, D, F = 1, 2048, 640, 1728
    return {
        "x": _w((lambda *s: _rng.normal(s) * 0.05)(B, S, D)),
        "w_gate": _w((lambda *s: _rng.normal(s) * 0.05)(D, F) * (D ** -0.5)),
        "w_up": _w((lambda *s: _rng.normal(s) * 0.05)(D, F) * (D ** -0.5)),
        "w_down": _w((lambda *s: _rng.normal(s) * 0.05)(F, D) * (F ** -0.5)),
    }

def reference(x, w_gate, w_up, w_down):
    g = jnp.einsum("bsd,df->bsf", x, w_gate)
    u = jnp.einsum("bsd,df->bsf", x, w_up)
    h = g * u
    return jnp.einsum("bsf,fd->bsd", h, w_down)
```

```python
import jax
import jax.numpy as jnp
from jax import lax
import jax.experimental.pallas as pl
import jax.experimental.pallas.tpu as pltpu

NT = (((1,), (1,)), ((), ()))
f32 = jnp.float32
bf16 = jnp.bfloat16
u32 = jnp.uint32

def dot_nt(a, b):
    return lax.dot_general(a, b, NT, preferred_element_type=f32)

def dot_nn(a, b):
    return jnp.dot(a, b, preferred_element_type=f32)

def make(xch=(128, 128, 256, 512), npre=2, nloop=2, sub=(384, 128), packed=True, split_first=True, semchk=False, store_bd=True, outsplit=True):
    S, D, F = 2048, 640, 1728
    HM = S // 2
    NP = 6
    H = NP * 128
    R0 = 2 * H
    KH = H + 128
    tm = HM // nloop
    assert sum(xch) == HM and sum(sub) == tm
    nx = len(xch)
    PK = 2 if packed else 1

    def rows(start, n, div=1, align=16):
        if isinstance(start, int):
            return pl.ds(start // div, n // div)
        return pl.ds(pl.multiple_of(start // div, align // div), n // div)

    def kern(x_hbm, wg_hbm, wu_hbm, wd_hbm, o_hbm, x_v, wg_v, wu_v, wr_v, wd_v, b0_v, bd_v, a_v, h_v, o_v, sem_x, sem_w, sem_o):
        def st(ref, idx, r0, n, c, val):
            val = val.astype(bf16)
            if packed:
                ref[idx, rows(r0, n, 2), c] = pltpu.bitcast(val, u32)
            else:
                ref[idx, rows(r0, n), c] = val
        def ld(ref, idx, r0, n, c=slice(None)):
            if packed:
                return pltpu.bitcast(ref[idx, rows(r0, n, 2), c], bf16)
            return ref[idx, rows(r0, n), c]

        def wcopy(src, dst, p, sem):
            return [pltpu.make_async_copy(src.at[pl.ds(o + 128 * p, 128)], dst.at[pl.ds(o + 128 * p, 128)], sem) for o in (0, H)]
        x_off = [sum(xch[:i]) for i in range(nx)]
        xc = [[pltpu.make_async_copy(x_hbm.at[pl.ds(o + x_off[i], xch[i])], x_v.at[pl.ds(o + x_off[i], xch[i])], sem_x.at[i]) for o in (0, HM)] for i in range(nx)]
        g0 = wcopy(wg_hbm, wg_v, 0, sem_x.at[0])
        u0 = wcopy(wu_hbm, wu_v, 0, sem_w.at[0] if split_first else sem_x.at[0])
        wp = [wcopy(wg_hbm, wg_v, p, sem_w.at[p]) + wcopy(wu_hbm, wu_v, p, sem_w.at[p]) for p in range(1, npre)]
        sem_r = sem_w.at[npre]
        n_rest = H - 128 * npre
        rest = []
        for src, dst in ((wg_hbm, wg_v), (wu_hbm, wu_v)):
            for o in (0, H):
                rest.append(pltpu.make_async_copy(src.at[pl.ds(o + 128 * npre, n_rest)], dst.at[pl.ds(o + 128 * npre, n_rest)], sem_r))
        for t in range(3):
            rest.append(pltpu.make_async_copy(wg_hbm.at[pl.ds(R0 + 64 * t, 64)], wr_v.at[pl.ds(128 * t, 64)], sem_r))
            rest.append(pltpu.make_async_copy(wu_hbm.at[pl.ds(R0 + 64 * t, 64)], wr_v.at[pl.ds(128 * t + 64, 64)], sem_r))
        rest += [
            pltpu.make_async_copy(wd_hbm.at[pl.ds(0, H)], wd_v.at[0, pl.ds(0, H)], sem_r),
            pltpu.make_async_copy(wd_hbm.at[pl.ds(H, H)], wd_v.at[1, pl.ds(0, H)], sem_r),
            pltpu.make_async_copy(wd_hbm.at[pl.ds(R0, 128)], wd_v.at[0, pl.ds(H, 128)], sem_r),
            pltpu.make_async_copy(wd_hbm.at[pl.ds(R0 + 128, 64)], wd_v.at[1, pl.ds(H, 64)], sem_r),
        ]
        def start(cs):
            for c in cs: c.start()
        def wait(cs):
            for c in cs: c.wait()

        def b_sums(w1, w2):
            b11 = w1[:, 0:256].astype(f32); b21 = w1[:, 256:512].astype(f32)
            b12 = w2[:, 0:256].astype(f32); b22 = w2[:, 256:512].astype(f32)
            return [(b11 + b22).astype(bf16), (b12 - b22).astype(bf16), (b21 - b11).astype(bf16),
                    (b11 + b12).astype(bf16), (b21 + b22).astype(bf16)]

        def a_sums(r0, n):
            rt = rows(r0, n); rb = rows(HM + r0, n)
            a11 = x_v[rt, 0:256].astype(f32); a12 = x_v[rt, 256:512].astype(f32)
            a21 = x_v[rb, 0:256].astype(f32); a22 = x_v[rb, 256:512].astype(f32)
            for k, v in enumerate((a11 + a22, a21 + a22, a11 + a12, a21 - a11, a12 - a22)):
                st(a_v, k, r0, n, slice(None), v)

        def strassen1(r0, n, w1, w2, bs):
            rt = rows(r0, n); rb = rows(HM + r0, n)
            t11 = dot_nt(x_v[rt, 512:640], w1[:, 512:640])
            t12 = dot_nt(x_v[rt, 512:640], w2[:, 512:640])
            t21 = dot_nt(x_v[rb, 512:640], w1[:, 512:640])
            t22 = dot_nt(x_v[rb, 512:640], w2[:, 512:640])
            m2 = dot_nt(ld(a_v, 1, r0, n), w1[:, 0:256])
            m5 = dot_nt(ld(a_v, 2, r0, n), w2[:, 256:512])
            c11 = t11 - m5; c12 = t12 + m5; c21 = t21 + m2; c22 = t22 - m2
            m1 = dot_nt(ld(a_v, 0, r0, n), bs[0])
            m3 = dot_nt(x_v[rt, 0:256], bs[1])
            c11 = c11 + m1; c12 = c12 + m3; c22 = c22 + (m1 + m3)
            m4 = dot_nt(x_v[rb, 256:512], bs[2])
            m6 = dot_nt(ld(a_v, 3, r0, n), bs[3])
            c11 = c11 + m4; c21 = c21 + m4; c22 = c22 + m6
            m7 = dot_nt(ld(a_v, 4, r0, n), bs[4])
            c11 = c11 + m7
            return c11, c12, c21, c22

        def h_sums(r0, n, c, h11, h12, h21, h22):
            for k, v in enumerate((h11 + h22, h21 + h22, h11, h22, h11 + h12, h21 - h11, h12 - h22)):
                st(h_v, k, r0, n, c, v)

        def tiles(w, p):
            return w[pl.ds(128 * p, 128), :], w[pl.ds(H + 128 * p, 128), :]

        def pair(p, r0, n):
            g = strassen1(r0, n, *tiles(wg_v, p), b_sums(*tiles(wg_v, p)))
            u = strassen1(r0, n, *tiles(wu_v, p), b_sums(*tiles(wu_v, p)))
            h_sums(r0, n, pl.ds(128 * p, 128), *[a * b for a, b in zip(g, u)])

        start(xc[0]); start(g0); start(u0); start(xc[1])
        wd_v[1, pl.ds(H + 64, 64), :] = jnp.zeros((64, D), bf16)
        for i in range(nx):
            r0, n = x_off[i], xch[i]
            wait(xc[i])
            if i == 0:
                wait(g0)
                if not split_first: wait(u0)
            if i + 2 < nx: start(xc[i + 2])
            elif i + 2 == nx:
                for c in wp: start(c)
            elif i + 1 == nx:
                start(rest)
            a_sums(r0, n)
            if i == 0:
                bg = b_sums(*tiles(wg_v, 0))
                for k in range(5): st(b0_v, k, 0, 128, slice(None), bg[k])
            else:
                bg = [ld(b0_v, k, 0, 128) for k in range(5)]
            g = strassen1(r0, n, *tiles(wg_v, 0), bg)
            if i == 0:
                if split_first: wait(u0)
                bu = b_sums(*tiles(wu_v, 0))
                for k in range(5): st(b0_v, 5 + k, 0, 128, slice(None), bu[k])
            else:
                bu = [ld(b0_v, 5 + k, 0, 128) for k in range(5)]
            u = strassen1(r0, n, *tiles(wu_v, 0), bu)
            h_sums(r0, n, pl.ds(0, 128), *[a * b for a, b in zip(g, u)])
        for p in range(1, npre):
            wait(wp[p - 1])
            pair(p, 0, HM)
        wait(rest)

        def d_sums():
            d1 = wd_v[0]; d2 = wd_v[1]
            b11 = d1[:, 0:256].astype(f32); b12 = d1[:, 256:640].astype(f32)
            b21 = d2[:, 0:256].astype(f32); b22 = d2[:, 256:640].astype(f32)
            b13 = b12[:, 256:384]; b23 = b22[:, 256:384]
            return [b11 + b22[:, 0:256], b12 - b22, jnp.concatenate([b21 - b11, b23 - b13], axis=1),
                    b11 + b12[:, 0:256], b21 + b22[:, 0:256]]

        def block(i, carry):
            r0 = i * tm
            for p in range(npre, NP):
                pair(p, r0, tm)
            w1 = wr_v[pl.ds(0, 128), :]; w2 = wr_v[pl.ds(256, 128), :]; w3 = wr_v[pl.ds(128, 128), :]
            c = strassen1(r0, tm, w1, w2, b_sums(w1, w2))
            ct = dot_nt(x_v[rows(r0, tm), :], w3)
            cb = dot_nt(x_v[rows(HM + r0, tm), :], w3)
            gate = lambda t: t * pltpu.roll(t, 64, 1)
            lo = lax.broadcasted_iota(jnp.int32, (tm, 128), 1) < 64
            h_sums(r0, tm, pl.ds(H, 128), jnp.where(lo, gate(c[0]), gate(ct)), jnp.where(lo, gate(c[1]), 0.0),
                   jnp.where(lo, gate(c[2]), gate(cb)), jnp.where(lo, gate(c[3]), 0.0))
            bd = [v.astype(bf16) for v in d_sums()]
            wid = (256, 384, 384, 256, 256)
            if store_bd:
                for k in range(5): st(bd_v, k, 0, KH, pl.ds(0, wid[k]), bd[k])
            s0 = 0
            for n in sub:
                q0 = r0 + s0
                if store_bd:
                    bd = [ld(bd_v, k, 0, KH, pl.ds(0, wid[k])) for k in range(5)]
                rt = rows(q0, n); rb = rows(HM + q0, n)
                def put(r, c0, w, val):
                    o_v[r, pl.ds(c0, w)] = val.astype(bf16)
                    if outsplit:
                        pltpu.make_async_copy(o_v.at[r, pl.ds(c0, w)], o_hbm.at[r, pl.ds(c0, w)], sem_o).start()
                m3 = dot_nn(ld(h_v, 2, q0, n), bd[1])
                m5 = dot_nn(ld(h_v, 4, q0, n), wd_v[1, :, 256:640])
                put(rt, 256, 384, m3 + m5)
                m4 = dot_nn(ld(h_v, 3, q0, n), bd[2])
                m2 = dot_nn(ld(h_v, 1, q0, n), wd_v[0, :, 0:256])
                m2t = dot_nn(ld(h_v, 1, q0, n), wd_v[0, :, 512:640])
                put(rb, 0, 256, m2 + m4[:, 0:256])
                put(rb, 512, 128, m2t + m4[:, 256:384])
                m1 = dot_nn(ld(h_v, 0, q0, n), bd[0])
                m6 = dot_nn(ld(h_v, 5, q0, n), bd[3])
                put(rb, 256, 256, (m3[:, 0:256] - m2) + m1 + m6)
                m7 = dot_nn(ld(h_v, 6, q0, n), bd[4])
                put(rt, 0, 256, (m4[:, 0:256] - m5[:, 0:256]) + m1 + m7)
                if not outsplit:
                    pltpu.make_async_copy(o_v.at[rt], o_hbm.at[rt], sem_o).start()
                    pltpu.make_async_copy(o_v.at[rb], o_hbm.at[rb], sem_o).start()
                s0 += n
            return carry
        if nloop == 1:
            block(0, 0)
        else:
            lax.fori_loop(0, nloop, block, 0)
        pltpu.make_async_copy(o_v, o_hbm, sem_o).wait()

    @jax.jit
    def f(x, w_gate, w_up, w_down):
        B = x.shape[0]
        x2 = x.reshape(S, D)
        hbm = pl.BlockSpec(memory_space=pltpu.HBM)
        pdt = u32 if packed else bf16
        out = pl.pallas_call(
            kern,
            in_specs=[hbm] * 4,
            out_specs=hbm,
            out_shape=jax.ShapeDtypeStruct((S, D), x.dtype),
            scratch_shapes=[
                pltpu.VMEM((S, D), bf16), pltpu.VMEM((R0, D), bf16), pltpu.VMEM((R0, D), bf16), pltpu.VMEM((384, D), bf16),
                pltpu.VMEM((2, KH, D), bf16),
                pltpu.VMEM((10, 128 // PK, 256), pdt),
                pltpu.VMEM((5, KH // PK, 384), pdt),
                pltpu.VMEM((5, HM // PK, 256), pdt), pltpu.VMEM((7, HM // PK, KH), pdt), pltpu.VMEM((S, D), bf16),
                pltpu.SemaphoreType.DMA((nx,)), pltpu.SemaphoreType.DMA((npre + 1,)), pltpu.SemaphoreType.DMA(()),
            ],
            compiler_params=pltpu.CompilerParams(vmem_limit_bytes=100 * 1024 * 1024, disable_semaphore_checks=not semchk),
        )(x2, w_gate.T, w_up.T, w_down)
        return out.reshape(B, S, D)
    return f


_impl = make()


@jax.jit
def pallas_standalone__glu_gated_bilinear__prompt_kernel(x, w_gate, w_up, w_down):
    return _impl(x, w_gate, w_up, w_down)
```

```python
import re

import jax
import jax.numpy as jnp
import numpy as np
from jax import lax
import jax.experimental.pallas as pl
import jax.experimental.pallas.tpu as pltpu

_S, _D, _F = 2048, 640, 1728
_T = 128
_LABELS = _D // _T
_HALF = _S // 2
_F_MAIN = 10 * _T

_CHUNKS = (128, 256, 640)
_BLOCK = 512


def _ten_tile_scheme():
    out = {}
    for i in range(_LABELS):
        l, r = i, 5 + i
        others = [j for j in range(_LABELS) if j != i]
        out["P", l] = ([(1, 0, l)], [(1, 0, i), (-1, 1, i)], [(1, i, l)] + [(1, i, 5 + j) for j in others])
        out["Q", l] = ([(1, 0, l), (1, 1, l)], [(1, 1, i)], [(1, i, l)] + [(-1, j, l) for j in others])
        out["P", r] = ([(1, 1, r)], [(1, 0, i), (-1, 1, i)], [(-1, i, r)] + [(-1, i, j) for j in others])
        out["Q", r] = ([(1, 0, r), (1, 1, r)], [(1, 0, i)], [(1, i, r)] + [(-1, j, r) for j in others])
        for j in others:
            r = 5 + j
            out["R1", l, r] = ([(1, 0, l), (1, 1, r)], [(1, 0, j), (1, 1, i)], [(1, j, l), (1, i, r)])
            out["R2", l, r] = ([(1, 0, r), (-1, 0, l)], [(1, 0, i), (1, 0, j)], [(1, i, r)])
            out["R3", l, r] = ([(1, 1, l), (-1, 1, r)], [(1, 1, i), (1, 1, j)], [(1, j, l)])
    return out


def _parse(table, first_tile=0):
    sign = lambda s: -1 if s == "-" else 1
    out = []
    for entry in table.split():
        f, d, w = entry.split("|")
        out.append((
            [(sign(s), "TB".index(h), first_tile + int(c)) for s, h, c in re.findall(r"([+-]?)([TB])(\d)", f)],
            [(sign(s), "TB".index(h), int(k)) for s, h, k in re.findall(r"([+-]?)([TB])(\d)", d)],
            [(sign(s), int(k), first_tile + int(c)) for s, k, c in re.findall(r"([+-]?)(\d)(\d)", w)],
        ))
    return out


_N_EARLY, _TILES_EARLY = 28, 4
_SEVEN_FIRST = _parse("""
    B1|B4|41              T2+B1|T3+B0|32+01        T1-T5|T2+T3|21           T1-T2|T0+T3|01
    -B0|T2-B2|20+22+23    T0-T2|T0+T2|00           T0+B0|T2|20-00-10        T2+B0|T2+B0|22+00
    T3|T0|03              T0-T3|T1+T2|10           T0|T3|30                 T0|T4|40
    B2-B0|B0+B2|22        B0|B3|30                 B2-B4|B0+B1|12           B0|B4|40
    T1-T3|T1+T3|11        T1|T4|41                 T3+B1|T3+B1|33+11        T1+B1|T3|31-01-11-21
    B3-B1|B1+B3|33        B2-B1|B0+B3|32           B2-B6|B0+B4|42           B3-B6|B1+B4|43
    T3+B0|T2+B1|23+10     B3-B0|B1+B2|23           B3|B0|03                 T3+B3|B1|13-23-33-43
    T5|T0|05              T4-T5|T1+T2|24           T4|T4|44                 T4|T3|34
    B5-B4|B1+B2|15        B4|B4|44                 -B4|T1-B1|14+12+15       B4|B3|34
    T4+B4|T1|14-04-24     T2|T0-B0|02+04+00+01+06  T4-T2|T0+T1|04           T2+B4|T1+B0|12+04
    T5+B5|B2|25-15-35-45  -B1|T3-B3|31+32+33+35    B5-B1|B2+B3|35           T5+B1|T3+B2|35+21
    T2+B6|T4+B0|42+06     T6-T2|T0+T4|06           T2+B2|B0|02-12-22-32-42  T6+B6|T4|46-06-16-26
    T5+B4|T1+B2|15+24     T6-T5|T2+T4|26           T5+B6|T4+B2|45+26        T5|T2-B2|25+24+21+26
    T3|T1-B1|13+10+11+16  T6|T3|36                 T3+B6|T4+B1|43+16        T6-T3|T1+T4|16
    B5|B0|05              -B6|T4-B4|46+42+43+45    B5-B6|B2+B4|45           B6|B3|36
""")
_SEVEN = _parse("""
    T5-T6|T2+T3|25                 B1-T6-B6|T2-T0-B2|06-21        B6-B1|T2+B0-T0-B2|06     T1+B1-T6-B6|T2-T0|21
    T4-T0|T1-T2|20+23              T5+B0|T1-B4|15-40-41           T4+B0|T1-B2|14-20-23     T5-T0|T1-T4|40+41
    B5-B0|B1-B4|15                 B1-B0-B2|B4-B0-B1|41           B2-B4|B0-B4|44           B4-B0|B1-B2|14
    -B6-B2|B2-B4|46                T6+B5|T3+B2|16+25+36           B6-B5|B2+B3|16+36        T6+B6|B2|26+21+46-16-23-36
    T6+T3+B6+B3-T0-B0|T1+T2-T3|23  T0+B0|T1|10+11+20+23+30+40+41  T0-T3|T3-T1|30-23        B0-T6-B6-B3|T1+T2-T3-B2|23-16
    T1+B1-T3-B3|T3-T0|31           T1|T0|00+01+21+31              B3-B1|T3+B0-T0-B3|03     B1-T3-B3|T3-T0-B3|03-31
    T6+T2|T2-T4|22                 B2-T6|B2-T4|22+46              T2+T3|T3+T4|32           T6|T2-B2|06+26+25-16-22
    T3|T3-B3|03+30+33-32           B3-B0|B3-B1|16-13              T3+B0|B3-T1|30-13        B0-B6-B3|T1+T2+B3-T3-B1-B2|16
    T1-T0-T2|T4-T0-T1|12           T0-T1-B2|T4-B0-B1|12-41        T0-T1|T0+T1-B0-B1|00-12  T2+B2|T4|02+22+42-32
    B0|T1-B1|00-10-14-15-13        T1+B1-T0-B0|B0+B1|11+41        B1|B0|06+01+03-11        T0+B0-T1|B0+B1-T1|00+11
    T4|T2-B2|20+24+23              T2-T4|T0-T4|02-12              T4+B2|B0-T4|02-12-44     T4|T0-B0|04+02+05-12
    B2+B3|B3+B4|43                 B2|T4-B4|46+43-44-41-42        T3-B2|T4+B3|43-32        T3+B3|B3|13+31+33-43
    B5-B4|B0-B3|34                 T4+B4|B2|14+24                 T4+B5|B0-T3|05-34        T4+B4|B0|04+34+44
    T5+B5|B4|15+45                 T5-T4|T0-T3|05                 T5+B5|T3|05+35-25        -B5|T3-B3|16+36+34+35
    T5|T4-B4|40+41+45
""")
_FOUR = _parse("""
    B0|T2-B2|00-20-21-22        T0+B0|T2|10+20+23+30+40     T1|T3-B3|01+30+31+32                 T1+B1|B3|21+31-33
    T2|T1-B1|02+10+12+40+42     T2+B2|B1|11+12+13+22+32-40  T3|T4|43                             B3|B4|43
    T3|T0|00+03+13+33           B3|B0|02+03-01-23           T1|T4|11+41                          B1|B4|40+41+42
    T2+B0|T2-B1|22+32-10-40     B2-B0|B1-B2|-22-32          T0-T2|T1-T2|10+40                    B1-T2-B2|T1-T4-B1|40+42-11
    B2-B1|T1+B4-T4-B1|32+42     T1+B1-T2-B2|T1-T4|11        T1+B0|T2-B3|21-30-32                 T0-T1|T2-T3|-30-32
    B1-B0|B2-B3|21+40-32        T3-T0-B0|T2-B0-B2|00+23     T0-T3|T0+T2-B0-B2|00                 T3+B3-T0-B0|B0+B2|23
    T1+B1+B3|T0+B3-T3|01+33     B1+B3|T3+B0-T0-B3|01        T1+T3+B1+B3|T3-T0|33                 B3-T2-B2|T0+B1-T1|13-02
    B3-B2|T0+B1-T1-B0|02        T2+B2-T3-B3|T0-T1|13        T2+B2-T0-B1|T1+B2+B4-T4-B1-B3|40-32  T2-T0|T1+T3+B2+B4-T2-T4-B1-B3|32
    T2+B2-T0-B0|B1+B3-B2-B4|40
""", first_tile=10)


def _up_order(ten):
    order, used = [], {}
    for l, partners in enumerate(((1, 2, 3, 4), (2, 3, 4, 0), (3, 4, 0, 1), (0, 1, 2, 4), (0, 1, 2, 3))):
        for j in partners:
            order += [ten[name, l, 5 + j] for name in ("R3", "R2", "R1")]
            c = 5 + j if (j - l) % 5 > 2 else l
            used[c] = used.get(c, 0) + 1
            order.append(ten["PQ"[used[c] - 1], c])
    return order


def _down_order(products):
    chains = {}
    for ff, df, wf in products:
        chains.setdefault(tuple(sorted(df, key=lambda t: (t[2], t[1]))), []).append((ff, wf))

    def key(df):
        labels = sorted({k for _, _, k in df})
        halves = tuple(h for _, h, _ in df)
        if labels[0] < _LABELS - 1:
            return (labels[0], len(labels), labels[-1], halves)
        return (labels[0], -len(df), 0, halves)

    return [(df, sorted(chains[df], key=lambda p: -min(c for _, _, c in p[0]))) for df in sorted(chains, key=key)]


def _assert_exact(products, num_tiles):
    t = np.zeros((2, num_tiles, 2, _LABELS, _LABELS, num_tiles), np.int64)
    for ff, df, wf in products:
        for sf, hf, cf in ff:
            for sd, hd, kd in df:
                for sw, kw, cw in wf:
                    t[hf, cf, hd, kd, kw, cw] += sf * sd * sw
    for h in range(2):
        for c in range(num_tiles):
            for k in range(_LABELS):
                t[h, c, h, k, k, c] -= 1
    assert not t.any()


_TEN = _ten_tile_scheme()
_UP = _up_order(_TEN)
_GATE_EARLY = [_TEN["R3", 0, r] for r in (6, 7, 8, 9)]
_GATE_REST = [p for p in _UP if not any(p is e for e in _GATE_EARLY)]
_DOWN_PRODUCTS = list(_TEN.values()) + _FOUR
_DOWN = _down_order(_DOWN_PRODUCTS)
_assert_exact(_UP, 10)
_assert_exact(_GATE_EARLY + _GATE_REST, 10)
_assert_exact(_SEVEN_FIRST, 7)
_assert_exact(_SEVEN, 7)
_assert_exact([(ff, df, wf) for df, chain in _DOWN for ff, wf in chain], 14)
assert all(c < _TILES_EARLY for _, _, wf in _SEVEN_FIRST[:_N_EARLY] for _, _, c in wf)


def _signed_sum(terms):
    terms = sorted(terms, key=lambda t: -t[0])
    acc = terms[0][1] if terms[0][0] > 0 else -terms[0][1]
    for s, v in terms[1:]:
        acc = acc + v if s > 0 else acc - v
    return acc


def _rows(start, size):
    return pl.ds(start if isinstance(start, int) else pl.multiple_of(start, 16), size)


def _blk(k):
    return pl.ds(_T * k, _T)


def _weight_sum(tile, wf):
    if len(wf) == 1 and wf[0][0] > 0:
        return tile(*wf[0][1:])
    return _signed_sum([(s, tile(k, c).astype(jnp.float32)) for s, k, c in wf]).astype(jnp.bfloat16)


def _matmul(a, w, contract_w, in_quarters):
    dot = lambda lhs: lax.dot_general(lhs, w, (((1,), (contract_w,)), ((), ())), preferred_element_type=jnp.float32)
    if not in_quarters:
        return dot(a)
    q = a.shape[0] // 4
    return jnp.concatenate([dot(a[z * q:(z + 1) * q]) for z in range(4)], axis=0)


def _accumulate(acc, key, sign, value):
    if key not in acc:
        acc[key] = (sign, value)
        return
    old_sign, old = acc[key]
    old = old() if callable(old) else old
    if sign == old_sign:
        acc[key] = (sign, old + value)
    else:
        acc[key] = (1, old - value if old_sign > 0 else value - old)


def _take(acc, key):
    sign, value = acc.pop(key)
    return value if sign > 0 else -value


def _kernel(x_hbm, wg_hbm, wu_hbm, wd_hbm, o_hbm,
            x_v, wg_v, wu_v, wr_v, wd_v, h_v, hr_v, g_v, o_top_v, o_bot_v, fence_v, sems):
    f32, bf16 = jnp.float32, jnp.bfloat16
    o_v = (o_top_v, o_bot_v)
    starts = [sum(_CHUNKS[:i]) for i in range(len(_CHUNKS))]

    def fetch(src, dst, row, size, sem, dst_row=None):
        dst_row = row if dst_row is None else dst_row
        return pltpu.make_async_copy(src.at[pl.ds(row, size)], dst.at[pl.ds(dst_row, size)], sems.at[sem])

    def fetch_x(i, sem):
        return [fetch(x_hbm, x_v, h * _HALF + starts[i], _CHUNKS[i], sem) for h in range(2)]

    def fetch_mixed_tiles(tiles, sem):
        return [fetch(w, wr_v, _F_MAIN + 64 * t, 64, sem, _T * t + 64 * q)
                for t in tiles for q, w in enumerate((wg_hbm, wu_hbm))]

    load_x0 = fetch_mixed_tiles(range(_TILES_EARLY), 0) + fetch_x(0, 0)
    load_tiles = fetch_mixed_tiles(range(_TILES_EARLY, 7), 1)
    load_x1 = fetch_x(1, 2)
    load_x2 = fetch_x(2, 3) + [fetch(wg_hbm, wg_v, 0, _T, 3)]
    load_rest = [fetch(wg_hbm, wg_v, _T, _F_MAIN - _T, 4), fetch(wu_hbm, wu_v, 0, _F_MAIN, 4),
                 fetch(wd_hbm, wd_v, 0, _F, 4)]
    for copy in load_x0 + load_tiles + load_x1 + load_x2 + load_rest:
        copy.start()

    def wait_all(copies):
        for copy in copies:
            copy.wait()

    wd_v[pl.ds(_F, 14 * _T - _F), :] = jnp.zeros((14 * _T - _F, _D), bf16)

    def fence():
        fence_v[...] = jnp.zeros(fence_v.shape, f32)

    def up_project(order, row, size, w_v, done, acc=None, before=None):
        tile = lambda k, c: w_v[_blk(c), _blk(k)]
        x_blk = lambda h, k: x_v[_rows(row + h * _HALF, size), _blk(k)]
        last = {(h, c): q for q, p in enumerate(order) for _, h, c in p[0]}
        acc = {} if acc is None else acc
        for q, (ff, df, wf) in enumerate(order):
            if before is not None:
                before(q)
            fence()
            if all(s < 0 for s, _, _ in wf):
                ff, wf = [(-s, h, c) for s, h, c in ff], [(-s, k, c) for s, k, c in wf]
            if len(df) == 1 and df[0][0] > 0:
                a = x_blk(*df[0][1:])
            else:
                a = _signed_sum([(s, x_blk(h, k).astype(f32)) for s, h, k in df]).astype(bf16)
            m = _matmul(a, _weight_sum(tile, wf), 1, q >= len(order) // 4 * 4)
            for s, h, c in ff:
                _accumulate(acc, (h, c), s, m)
                if done is not None and last[h, c] == q:
                    done(h, c, _take(acc, (h, c)), q)
        return acc

    deferred = []
    for i, (row, size, loads) in enumerate(zip(starts, _CHUNKS, (load_x0, load_x1, load_x2))):
        wait_all(loads)
        for fn in deferred:
            fn()
        deferred = []
        order = _SEVEN_FIRST if i == 0 else _SEVEN
        have = {}

        def gate(h, c, row=row, size=size, have=have):
            low = lax.broadcasted_iota(jnp.int32, (size, _T), 1) < 64
            if c == 6:
                v = jnp.where(low, have[h, c] * pltpu.roll(have[h, c], 64, 1), 0.0)
            else:
                a, b = have[h, c & ~1], have[h, c | 1]
                v = jnp.where(low, a, b) * pltpu.roll(jnp.where(low, b, a), 64, 1)
            hr_v[_rows(row + h * _HALF, size), _blk(c // 2)] = v

        def done(h, c, v, q, i=i, order=order, have=have, gate=gate):
            have[h, c] = v
            if c == 6 or (h, c ^ 1) in have:
                if q >= len(order) - 5 and i + 1 < len(_CHUNKS):
                    deferred.append(lambda: gate(h, c))
                else:
                    gate(h, c)

        def before(q, i=i):
            if i == 0 and q == _N_EARLY:
                wait_all(load_tiles)

        up_project(order, row, size, wr_v, done, before=before)

    early_slots = {}
    for row, size in ((starts[-1], _CHUNKS[-1]), (0, starts[-1])):
        for slot, (key, (sign, v)) in enumerate(up_project(_GATE_EARLY, row, size, wg_v, None).items()):
            g_v[slot, _rows(row, size), :] = v
            early_slots[key] = (sign, slot)
    wait_all(load_rest)

    def block(i, carry):
        row = i * _BLOCK
        g = {}

        def done_gate(h, c, v, q):
            g[h, c] = v

        def done_up(h, c, v, q):
            h_v[_rows(h * _BLOCK, _BLOCK), _blk(c)] = g[h, c] * v

        early = {key: (sign, lambda slot=slot: g_v[slot, _rows(row, _BLOCK), :])
                 for key, (sign, slot) in early_slots.items()}
        up_project(_GATE_REST, row, _BLOCK, wg_v, done_gate, acc=early)
        up_project(_UP, row, _BLOCK, wu_v, done_up)

        def h_blk(h, c):
            if c >= 10:
                return hr_v[_rows(row + h * _HALF, _BLOCK), _blk(c - 10)]
            return h_v[_rows(h * _BLOCK, _BLOCK), _blk(c)]

        tile = lambda k, c: wd_v[_blk(c), _blk(k)]
        last = {(h, k): q for q, (df, _) in enumerate(_DOWN) for _, h, k in df}
        acc, count = {}, 0
        for q, (df, chain) in enumerate(_DOWN):
            m = None
            for ff, wf in chain:
                fence()
                a = _signed_sum([(s, h_blk(h, c)) for s, h, c in ff]).astype(bf16)
                d = _matmul(a, _weight_sum(tile, wf), 0, count >= len(_DOWN_PRODUCTS) // 4 * 4)
                m = d if m is None else m + d
                count += 1
            for s, h, k in df:
                _accumulate(acc, (h, k), s, m)
                if last[h, k] == q:
                    v = _take(acc, (h, k))
                    step = _BLOCK // 4 if k == _LABELS - 1 else _BLOCK
                    for z in range(0, _BLOCK, step):
                        r = _rows(row + z, step)
                        o_v[h][r, _blk(k)] = v[z:z + step].astype(bf16)
                        pltpu.make_async_copy(o_v[h].at[r, _blk(k)],
                                              o_hbm.at[_rows(row + h * _HALF + z, step), _blk(k)],
                                              sems.at[h]).start()
        return carry

    lax.fori_loop(0, _HALF // _BLOCK, block, 0)
    for h in range(2):
        pltpu.make_async_copy(o_v[h], o_hbm.at[pl.ds(h * _HALF, _HALF)], sems.at[h]).wait()


@jax.jit
def pallas_standalone__glu_gated_bilinear__prompt_kernel(
    x: jax.Array,
    w_gate: jax.Array,
    w_up: jax.Array,
    w_down: jax.Array,
):
    assert x.shape == (1, _S, _D) and w_gate.shape == w_up.shape == (_D, _F) and w_down.shape == (_F, _D)
    f32, bf16 = jnp.float32, jnp.bfloat16
    hbm = pl.BlockSpec(memory_space=pltpu.HBM)
    out = pl.pallas_call(
        _kernel,
        in_specs=[hbm] * 4,
        out_specs=hbm,
        out_shape=jax.ShapeDtypeStruct((_S, _D), bf16),
        scratch_shapes=[
            pltpu.VMEM((_S, _D), bf16),
            pltpu.VMEM((_F_MAIN, _D), bf16),
            pltpu.VMEM((_F_MAIN, _D), bf16),
            pltpu.VMEM((7 * _T, _D), bf16),
            pltpu.VMEM((14 * _T, _D), bf16),
            pltpu.VMEM((2 * _BLOCK, _F_MAIN), f32),
            pltpu.VMEM((_S, 4 * _T), f32),
            pltpu.VMEM((5, _HALF, _T), f32),
            pltpu.VMEM((_HALF, _D), bf16),
            pltpu.VMEM((_HALF, _D), bf16),
            pltpu.VMEM((8, _T), f32),
            pltpu.SemaphoreType.DMA((5,)),
        ],
        compiler_params=pltpu.CompilerParams(vmem_limit_bytes=100 * 1024 * 1024),
    )(x.reshape(_S, _D), w_gate.T, w_up.T, w_down)
    return out.reshape(x.shape)
```

```python
import re

import jax
import jax.numpy as jnp
import numpy as np
from jax import lax
import jax.experimental.pallas as pl
import jax.experimental.pallas.tpu as pltpu

_S, _D, _F = 2048, 640, 1728
_T = 128
_LABELS = _D // _T
_HALF = _S // 2
_F_MAIN = 10 * _T

_CHUNKS = (192, 192, 320, 320)
_TILE_GROUPS = ((0, 1), (2,), (3,), (4,), (5,), (6,))
_BLOCK = 512


def _ten_tile_scheme():
    out = {}
    for i in range(_LABELS):
        l, r = i, 5 + i
        others = [j for j in range(_LABELS) if j != i]
        out["P", l] = ([(1, 0, l)], [(1, 0, i), (-1, 1, i)], [(1, i, l)] + [(1, i, 5 + j) for j in others])
        out["Q", l] = ([(1, 0, l), (1, 1, l)], [(1, 1, i)], [(1, i, l)] + [(-1, j, l) for j in others])
        out["P", r] = ([(1, 1, r)], [(1, 0, i), (-1, 1, i)], [(-1, i, r)] + [(-1, i, j) for j in others])
        out["Q", r] = ([(1, 0, r), (1, 1, r)], [(1, 0, i)], [(1, i, r)] + [(-1, j, r) for j in others])
        for j in others:
            r = 5 + j
            out["R1", l, r] = ([(1, 0, l), (1, 1, r)], [(1, 0, j), (1, 1, i)], [(1, j, l), (1, i, r)])
            out["R2", l, r] = ([(1, 0, r), (-1, 0, l)], [(1, 0, i), (1, 0, j)], [(1, i, r)])
            out["R3", l, r] = ([(1, 1, l), (-1, 1, r)], [(1, 1, i), (1, 1, j)], [(1, j, l)])
    return out


def _parse(table, first_tile=0):
    sign = lambda s: -1 if s == "-" else 1
    out = []
    for entry in table.split():
        f, d, w = entry.split("|")
        out.append((
            [(sign(s), "TB".index(h), first_tile + int(c)) for s, h, c in re.findall(r"([+-]?)([TB])(\d)", f)],
            [(sign(s), "TB".index(h), int(k)) for s, h, k in re.findall(r"([+-]?)([TB])(\d)", d)],
            [(sign(s), int(k), first_tile + int(c)) for s, k, c in re.findall(r"([+-]?)(\d)(\d)", w)],
        ))
    return out


_SEVEN_FIRST = _parse("""
    B0|B4|40                 T0-T1|T1+T2|20           B0|B3|30               T0+B0|T1|10-00-20
    T0|T4|40                 T0|T3|30                 T0-T2|T0+T1|00         B1-B3|B2+B3|31
    T1|T0|01                 T1+B0|T1+B2|11+20        B1-B0|B1+B2|11         T1+B1|B2|21-11-31-41
    B1-B4|B2+B4|41           B1|B0|01                 B2-B3|B0+B3|32         B2-B4|B0+B4|42
    T2+B2|B0|02-12-22-32-42  B2-B6|B0+B2|22           B2-B0|B0+B1|12         T2+B0|T1+B0|12+00
    -B0|T1-B1|10+12+11       T3|T4|43                 T3-T2|T0+T3|03         T3-T1|T2+T3|23
    T3+B3|T3|33-03-13-23     T3-T5|T1+T3|13           T1+B3|T3+B2|31+23      B3|B4|43
    T2+B3|T3+B0|32+03        T2+B4|T4+B0|42+04        T4-T2|T0+T4|04         T4+B4|T4|44-04-14-24
    T1+B4|T4+B2|41+24        B4|B3|34                 T1|T2-B2|21+20+23+24   T4-T1|T2+T4|24
    T4|T3|34                 T4-T5|T1+T4|14           T5+B3|T3+B1|35+13      -B3|T3-B3|33+32+35+31
    T5+B5|B1|15-25-35-45     B5|B0|05                 B5-B3|B1+B3|35         B5-B6|B1+B2|25
    T5+B4|T4+B1|45+14        T5|T0|05                 -B4|T4-B4|44+42+45+41  B5-B4|B1+B4|45
    T6-T2|T0+T2|06           T2|T0-B0|02+00+06+03+04  T2+B6|T2+B0|22+06      T6|T4|46
    -B6|T2-B2|26+22+25       T6|T3|36                 T6+B6|T2|26-06-16      B6|B3|36
    T5|T1-B1|15+16+13+14     T6-T5|T1+T2|16           T5+B6|T2+B1|25+16      B6|B4|46
""")
_SEVEN = _parse("""
    T5-T6|T1-T4|46+40              T5-T2|T2+T3|25                 T2+T3|T2-T4|23                 T3+T1|T3+T4|33
    T6-T1|T3-T1|36-21              T2+T1+B2+B1-T6-B6|T1+T2-T3|21  T2+B2|B2|22+20+42-12-21-32     T1+B6|B3-T1|36-11
    T4+B6|T1-B2|14-26-21           T6+B6|T1|16+10+26+21+36+46+40  T4-T6|T1-T2|26+21              T5+B6|T1-B4|15-46-40
    T6-T0-B3|T4-B0-B1|13-40        T0+B0-T6-B6|B0+B1|10+40        B0|B0|02+00+01-10              B0-B6-B3|B4-B0-B1|40
    B0-T2-B2|T2-T0-B2|02-20        B2-B0|T2+B0-T0-B2|02           T0+B0-T2-B2|T2-T0|20           T2|T2-B2|02+22+25-12-23
    -B5|T3-B3|12+32+34+35          T2+B5|T3+B2|12+25+32           B4-B6|B1-B2|14                 B5-B6|B1-B4|15
    B6-T2-B2-B1|T1+T2-T3-B2|21-12  B6|T1-B1|06-16-14-15-11        B6-B2-B1|T1+T2+B3-T3-B1-B2|12  B1-B6|B3-B1|12-11
    T0|T0|06+00+20+30              T0-T6-T3|T4-T0-T1|13           T6+B6-T0|B0+B1-T1|06+10        T6-T0|T0+T1-B0-B1|06-13
    T4+B3|B0-T4|03-13-44           B3-T2|B2-T4|23+42              T3-T4|T0-T4|03-13              T3+B3|T4|03+23+43-33
    T0+B0-T1-B1|T3-T0|30           B0-T1-B1|T3-T0-B3|01-30        B1-B0|T3+B0-T0-B3|01           T1|T3-B3|01+36+31-33
    B3|T4-B4|42+41-44-40-43        T1-B3|T4+B3|41-33              T1+B1|B3|11+30+31-41           B3+B1|B3+B4|41
    B2-B5|B2+B3|12+32              B5-B4|B0-B3|34                 B3-B4|B0-B4|44                 -B2-B3|B2-B4|42
    T5-T4|T0-T3|05                 T5+B5|B4|15+45                 T5+B5|T3|05+35-25              T4+B5|B0-T3|05-34
    T4+B4|B2|14+24                 T4+B4|B0|04+34+44              T4|T2-B2|26+24+21              T4|T0-B0|04+03+05-13
    T5|T4-B4|46+40+45
""")
_FOUR = _parse("""
    B0|T2-B2|00-20-21-22        T0+B0|T2|10+20+23+30+40     T1|T3-B3|01+30+31+32                 T1+B1|B3|21+31-33
    T2|T1-B1|02+10+12+40+42     T2+B2|B1|11+12+13+22+32-40  T3|T4|43                             B3|B4|43
    T3|T0|00+03+13+33           B3|B0|02+03-01-23           T1|T4|11+41                          B1|B4|40+41+42
    T2+B0|T2-B1|22+32-10-40     B2-B0|B1-B2|-22-32          T0-T2|T1-T2|10+40                    B1-T2-B2|T1-T4-B1|40+42-11
    B2-B1|T1+B4-T4-B1|32+42     T1+B1-T2-B2|T1-T4|11        T1+B0|T2-B3|21-30-32                 T0-T1|T2-T3|-30-32
    B1-B0|B2-B3|21+40-32        T3-T0-B0|T2-B0-B2|00+23     T0-T3|T0+T2-B0-B2|00                 T3+B3-T0-B0|B0+B2|23
    T1+B1+B3|T0+B3-T3|01+33     B1+B3|T3+B0-T0-B3|01        T1+T3+B1+B3|T3-T0|33                 B3-T2-B2|T0+B1-T1|13-02
    B3-B2|T0+B1-T1-B0|02        T2+B2-T3-B3|T0-T1|13        T2+B2-T0-B1|T1+B2+B4-T4-B1-B3|40-32  T2-T0|T1+T3+B2+B4-T2-T4-B1-B3|32
    T2+B2-T0-B0|B1+B3-B2-B4|40
""", first_tile=10)


def _up_order(ten):
    order, used = [], {}
    for l, partners in enumerate(((1, 2, 3, 4), (2, 3, 4, 0), (3, 4, 0, 1), (0, 1, 2, 4), (0, 1, 2, 3))):
        for j in partners:
            order += [ten[name, l, 5 + j] for name in ("R3", "R2", "R1")]
            c = 5 + j if (j - l) % 5 > 2 else l
            used[c] = used.get(c, 0) + 1
            order.append(ten["PQ"[used[c] - 1], c])
    return order


def _down_order(products):
    chains = {}
    for ff, df, wf in products:
        chains.setdefault(tuple(sorted(df, key=lambda t: (t[2], t[1]))), []).append((ff, wf))

    def key(df):
        labels = sorted({k for _, _, k in df})
        halves = tuple(h for _, h, _ in df)
        if labels[0] < _LABELS - 1:
            return (labels[0], len(labels), labels[-1], halves)
        return (labels[0], -len(df), 0, halves)

    return [(df, sorted(chains[df], key=lambda p: -min(c for _, _, c in p[0]))) for df in sorted(chains, key=key)]


def _assert_exact(products, num_tiles):
    t = np.zeros((2, num_tiles, 2, _LABELS, _LABELS, num_tiles), np.int64)
    for ff, df, wf in products:
        for sf, hf, cf in ff:
            for sd, hd, kd in df:
                for sw, kw, cw in wf:
                    t[hf, cf, hd, kd, kw, cw] += sf * sd * sw
    for h in range(2):
        for c in range(num_tiles):
            for k in range(_LABELS):
                t[h, c, h, k, k, c] -= 1
    assert not t.any()


_TEN = _ten_tile_scheme()
_UP = _up_order(_TEN)
_EARLY_TILES = 3
_GATE_EARLY = [_TEN["R3", l, 5 + j] for l in range(_EARLY_TILES) for j in range(_LABELS) if j != l]
_GATE_REST = [p for p in _UP if not any(p is e for e in _GATE_EARLY)]
_EARLY_BLOCKS = sorted({(h, c) for ff, _, _ in _GATE_EARLY for _, h, c in ff})
_DOWN_PRODUCTS = list(_TEN.values()) + _FOUR
_DOWN = _down_order(_DOWN_PRODUCTS)
_assert_exact(_UP, 10)
_assert_exact(_GATE_EARLY + _GATE_REST, 10)
assert all(c < _EARLY_TILES for _, _, wf in _GATE_EARLY for _, _, c in wf)
_assert_exact(_SEVEN_FIRST, 7)
_assert_exact(_SEVEN, 7)
_assert_exact([(ff, df, wf) for df, chain in _DOWN for ff, wf in chain], 14)


def _signed_sum(terms):
    terms = sorted(terms, key=lambda t: -t[0])
    acc = terms[0][1] if terms[0][0] > 0 else -terms[0][1]
    for s, v in terms[1:]:
        acc = acc + v if s > 0 else acc - v
    return acc


def _rows(start, size):
    return pl.ds(start if isinstance(start, int) else pl.multiple_of(start, 16), size)


def _blk(k):
    return pl.ds(_T * k, _T)


def _weight_sum(tile, wf):
    if len(wf) == 1 and wf[0][0] > 0:
        return tile(*wf[0][1:])
    return _signed_sum([(s, tile(k, c).astype(jnp.float32)) for s, k, c in wf]).astype(jnp.bfloat16)


def _matmul(a, w, contract_w, in_quarters):
    dot = lambda lhs: lax.dot_general(lhs, w, (((1,), (contract_w,)), ((), ())), preferred_element_type=jnp.float32)
    if not in_quarters:
        return dot(a)
    q = a.shape[0] // 4
    return jnp.concatenate([dot(a[z * q:(z + 1) * q]) for z in range(4)], axis=0)


def _accumulate(acc, key, sign, value):
    if key not in acc:
        acc[key] = (sign, value)
        return
    old_sign, old = acc[key]
    old = old() if callable(old) else old
    if sign == old_sign:
        acc[key] = (sign, old + value)
    else:
        acc[key] = (1, old - value if old_sign > 0 else value - old)


def _take(acc, key):
    sign, value = acc.pop(key)
    return value if sign > 0 else -value


def _kernel(x_hbm, wg_hbm, wu_hbm, wd_hbm, o_hbm,
            x_v, wg_v, wu_v, wr_v, wd_v, h_v, hr_v, g_v, o_top_v, o_bot_v, fence_v, sems):
    f32, bf16 = jnp.float32, jnp.bfloat16
    o_v = (o_top_v, o_bot_v)
    starts = [sum(_CHUNKS[:i]) for i in range(len(_CHUNKS))]

    wd_v[pl.ds(_F, 14 * _T - _F), :] = jnp.zeros((14 * _T - _F, _D), bf16)

    def fetch(src, dst, row, size, sem, dst_row=None):
        dst_row = row if dst_row is None else dst_row
        return pltpu.make_async_copy(src.at[pl.ds(row, size)], dst.at[pl.ds(dst_row, size)], sems.at[sem])

    def fetch_x(i, sem):
        return [fetch(x_hbm, x_v, h * _HALF + starts[i], _CHUNKS[i], sem) for h in range(2)]

    def fetch_mixed_tiles(tiles, sem):
        return [fetch(w, wr_v, _F_MAIN + 64 * t, 64, sem, _T * t + 64 * q)
                for t in tiles for q, w in enumerate((wg_hbm, wu_hbm))]

    n_groups, n_chunks = len(_TILE_GROUPS), len(_CHUNKS)
    sem_rest = n_groups + n_chunks - 1
    load_tiles = [fetch_mixed_tiles(tiles, q) for q, tiles in enumerate(_TILE_GROUPS)]
    load_x = [fetch_x(i, n_groups + i - 1 if i else 0) for i in range(n_chunks)]
    load_x[0] += load_tiles.pop(0)
    load_x[-1].append(fetch(wg_hbm, wg_v, 0, _EARLY_TILES * _T, sem_rest - 1))
    load_rest = [fetch(wg_hbm, wg_v, _EARLY_TILES * _T, _F_MAIN - _EARLY_TILES * _T, sem_rest),
                 fetch(wu_hbm, wu_v, 0, _F_MAIN, sem_rest), fetch(wd_hbm, wd_v, 0, _F, sem_rest)]
    for copies in load_x[:1] + load_tiles + load_x[1:] + [load_rest]:
        for copy in copies:
            copy.start()

    def wait_all(copies):
        for copy in copies:
            copy.wait()

    def fence():
        fence_v[...] = jnp.zeros(fence_v.shape, f32)

    def up_project(order, row, size, w_v, done, acc=None, before=None):
        tile = lambda k, c: w_v[_blk(c), _blk(k)]
        x_blk = lambda h, k: x_v[_rows(row + h * _HALF, size), _blk(k)]
        last = {(h, c): q for q, p in enumerate(order) for _, h, c in p[0]}
        acc = {} if acc is None else acc
        for q, (ff, df, wf) in enumerate(order):
            if before is not None:
                before(q)
            fence()
            if all(s < 0 for s, _, _ in wf):
                ff, wf = [(-s, h, c) for s, h, c in ff], [(-s, k, c) for s, k, c in wf]
            if len(df) == 1 and df[0][0] > 0:
                a = x_blk(*df[0][1:])
            else:
                a = _signed_sum([(s, x_blk(h, k).astype(f32)) for s, h, k in df]).astype(bf16)
            m = _matmul(a, _weight_sum(tile, wf), 1, q >= len(order) // 4 * 4)
            for s, h, c in ff:
                _accumulate(acc, (h, c), s, m)
                if done is not None and last[h, c] == q:
                    done(h, c, _take(acc, (h, c)))
        return acc

    for i, (row, size) in enumerate(zip(starts, _CHUNKS)):
        wait_all(load_x[i])
        order = _SEVEN_FIRST if i == 0 else _SEVEN
        have = {}

        def done(h, c, v, row=row, size=size, have=have):
            have[h, c] = v
            low = lax.broadcasted_iota(jnp.int32, (size, _T), 1) < 64
            if c == 6:
                v = jnp.where(low, v * pltpu.roll(v, 64, 1), 0.0)
            elif (h, c ^ 1) in have:
                a, b = have[h, c & ~1], have[h, c | 1]
                v = jnp.where(low, a, b) * pltpu.roll(jnp.where(low, b, a), 64, 1)
            else:
                return
            hr_v[_rows(row + h * _HALF, size), _blk(c // 2)] = v

        def before(q, order=order):
            while load_tiles and _TILE_GROUPS[n_groups - len(load_tiles)][0] <= max(c for _, _, c in order[q][2]):
                wait_all(load_tiles.pop(0))

        up_project(order, row, size, wr_v, done, before=before)

    early_sign = {}
    for row, size in zip(starts, _CHUNKS):
        for key, (sign, v) in up_project(_GATE_EARLY, row, size, wg_v, None).items():
            g_v[_EARLY_BLOCKS.index(key), _rows(row, size), :] = v
            early_sign[key] = sign
    wait_all(load_rest)

    def block(i, carry):
        row = i * _BLOCK
        g = {}

        def done_gate(h, c, v):
            g[h, c] = v

        def done_up(h, c, v):
            h_v[_rows(h * _BLOCK, _BLOCK), _blk(c)] = g[h, c] * v

        early = {key: (early_sign[key], lambda slot=slot: g_v[slot, _rows(row, _BLOCK), :])
                 for slot, key in enumerate(_EARLY_BLOCKS)}
        up_project(_GATE_REST, row, _BLOCK, wg_v, done_gate, acc=early)
        up_project(_UP, row, _BLOCK, wu_v, done_up)

        def h_blk(h, c):
            if c >= 10:
                return hr_v[_rows(row + h * _HALF, _BLOCK), _blk(c - 10)]
            return h_v[_rows(h * _BLOCK, _BLOCK), _blk(c)]

        tile = lambda k, c: wd_v[_blk(c), _blk(k)]
        last = {(h, k): q for q, (df, _) in enumerate(_DOWN) for _, h, k in df}
        acc, count = {}, 0
        for q, (df, chain) in enumerate(_DOWN):
            m = None
            for ff, wf in chain:
                fence()
                a = _signed_sum([(s, h_blk(h, c)) for s, h, c in ff]).astype(bf16)
                d = _matmul(a, _weight_sum(tile, wf), 0, count >= len(_DOWN_PRODUCTS) // 4 * 4)
                m = d if m is None else m + d
                count += 1
            for s, h, k in df:
                _accumulate(acc, (h, k), s, m)
                if last[h, k] == q:
                    v = _take(acc, (h, k))
                    step = _BLOCK // 4 if k == _LABELS - 1 else _BLOCK
                    for z in range(0, _BLOCK, step):
                        r = _rows(row + z, step)
                        o_v[h][r, _blk(k)] = v[z:z + step].astype(bf16)
                        pltpu.make_async_copy(o_v[h].at[r, _blk(k)],
                                              o_hbm.at[_rows(row + h * _HALF + z, step), _blk(k)],
                                              sems.at[h]).start()
        return carry

    lax.fori_loop(0, _HALF // _BLOCK, block, 0)
    for h in range(2):
        pltpu.make_async_copy(o_v[h], o_hbm.at[pl.ds(h * _HALF, _HALF)], sems.at[h]).wait()


@jax.jit
def pallas_standalone__glu_gated_bilinear__prompt_kernel(
    x: jax.Array,
    w_gate: jax.Array,
    w_up: jax.Array,
    w_down: jax.Array,
):
    assert x.shape == (1, _S, _D) and w_gate.shape == w_up.shape == (_D, _F) and w_down.shape == (_F, _D)
    f32, bf16 = jnp.float32, jnp.bfloat16
    hbm = pl.BlockSpec(memory_space=pltpu.HBM)
    out = pl.pallas_call(
        _kernel,
        in_specs=[hbm] * 4,
        out_specs=hbm,
        out_shape=jax.ShapeDtypeStruct((_S, _D), bf16),
        scratch_shapes=[
            pltpu.VMEM((_S, _D), bf16),
            pltpu.VMEM((_F_MAIN, _D), bf16),
            pltpu.VMEM((_F_MAIN, _D), bf16),
            pltpu.VMEM((7 * _T, _D), bf16),
            pltpu.VMEM((14 * _T, _D), bf16),
            pltpu.VMEM((2 * _BLOCK, _F_MAIN), f32),
            pltpu.VMEM((_S, 4 * _T), f32),
            pltpu.VMEM((len(_EARLY_BLOCKS), _HALF, _T), f32),
            pltpu.VMEM((_HALF, _D), bf16),
            pltpu.VMEM((_HALF, _D), bf16),
            pltpu.VMEM((8, _T), f32),
            pltpu.SemaphoreType.DMA((len(_TILE_GROUPS) + len(_CHUNKS),)),
        ],
        compiler_params=pltpu.CompilerParams(
            vmem_limit_bytes=100 * 1024 * 1024,
            flags={"XLA_TPU_RESCHEDULE_DMA_DONES": True},
        ),
    )(x.reshape(_S, _D), w_gate.T, w_up.T, w_down)
    return out.reshape(x.shape)
```
